```python
import os as _os
_os.environ.setdefault("JAX_PLATFORMS", "cpu")
import jax
import jax.numpy as jnp

def _softmax(x, axis=-1):
    return jax.nn.softmax(x, axis=axis)
def _gelu(x):
    return jax.nn.gelu(x, approximate=True)
def _silu(x):
    return jax.nn.silu(x)
def _sigmoid(x):
    return jax.nn.sigmoid(x)
def _layernorm(x, axis=-1, eps=1e-5):
    m = jnp.mean(x, axis=axis, keepdims=True)
    v = jnp.var(x, axis=axis, keepdims=True)
    return (x - m) / jnp.sqrt(v + eps)
def _scatter_add(tgt, idx, src, axis=0):
    return tgt.at[idx].add(src)
def _segment_sum(src, seg, n):
    return jax.ops.segment_sum(src, seg, n)
class _Rng:
    def __init__(self, key):
        self._k = key
    def _next(self):
        self._k, sub = jax.random.split(self._k)
        return sub
    def normal(self, shape):
        return jax.random.normal(self._next(), shape, dtype=jnp.bfloat16)
    def randint(self, lo, hi, shape):
        return jax.random.randint(self._next(), shape, lo, hi, dtype=jnp.int32)
    def uniform(self, shape, lo=0.0, hi=1.0):
        return jax.random.uniform(self._next(), shape, jnp.bfloat16, lo, hi)
    def permutation(self, n):
        return jax.random.permutation(self._next(), n)


kernel_name = 'standalone__mixer_token_mlp__sampling'

def setup_inputs():
    _rng = _Rng(jax.random.key(int.from_bytes(__import__("os").urandom(4), "little")))
    _w = (lambda a: (lambda t: t.astype(jnp.bfloat16) if jnp.issubdtype(t.dtype, jnp.floating) else t)(jnp.asarray(a)))
    B, S, D, F = 32, 16, 1024, 3584
    return {
        "x": _w((lambda *s: _rng.normal(s) * 0.05)(B, S, D)),
        "w1": _w((lambda *s: _rng.normal(s) * 0.05)(S, F) * (S ** -0.5)),
        "b1": _w((lambda *s: _rng.normal(s) * 0.05)(F) * 0.02),
        "w2": _w((lambda *s: _rng.normal(s) * 0.05)(F, S) * (F ** -0.5)),
        "b2": _w((lambda *s: _rng.normal(s) * 0.05)(S) * 0.02),
    }

def reference(x, w1, b1, w2, b2):
    B, S, D = x.shape
    h = _layernorm(x, axis=-1)
    u = jnp.einsum("bsd,sf->bdf", h, w1) + b1
    u = _gelu(u)
    y = jnp.einsum("bdf,fs->bds", u, w2) + b2
    return (lambda x, *d: x.transpose(*d))(y, 0, 2, 1)
```

```python
import numpy as np
import jax, jax.numpy as jnp
from jax import lax
import jax.experimental.pallas as pl
import jax.experimental.pallas.tpu as pltpu

C1 = float(np.sqrt(2.0 / np.pi))
C2 = C1 * 0.044715
SC = float(C2 ** (1.0 / 3.0))
KK = C1 / SC
f32, bf16, u32 = jnp.float32, jnp.bfloat16, jnp.uint32
LP = {'XLA_TPU_FORCE_LP_LLO_SCHEDULER': True}
ED = {'XLA_TPU_EVENLY_DISTRIBUTE_CRITICAL_NODES': True}
DN = (((1,), (0,)), ((), ()))

def make(U=2, flags=None, NIT=None, V=32, DL=11, PD=8, WM=3.0, VD=1, GP=11, GM=0xff, AM=0xff, TL=1, PH=0.0, AP=None, NL=2, CH=2, LP_=3, XS=8, HALF=0, ORD='gfz'):
    FC = 128
    DC = 512
    NT = DC // 128
    AP = AP or GP
    def act(w):
        return w * jnp.tanh(w * (w * w + KK))
    def kern(x_hbm, w1_hbm, b1_hbm, w2_hbm, b2_hbm, o_hbm, x_s, w1_s, b1_s, w2_s, b2_s, o_s, wb_s, hp_s, hf_s, idx_s, sem, *lss):
        S, F = w1_hbm.shape
        B, _, D = x_hbm.shape
        NK = F // FC
        NG = F // 8
        NC = D // DC
        UB = U // NC
        NA = (NG - V) // 2
        cps = [pltpu.make_async_copy(s, d, sem.at[i]) for i, (s, d) in enumerate(
            [(w1_hbm, w1_s), (b1_hbm, b1_s), (w2_hbm, w2_s), (b2_hbm, b2_s), (x_hbm.at[0:UB], x_s.at[0:UB]), (x_hbm.at[UB:], x_s.at[UB:])])]
        for c in cps[:5]: c.start()
        vpos = [2 * int((j + PH) * NA / V) + j for j in range(V)]
        mpos = [p for p in range(NG) if p not in vpos][0::2]
        R_M = F // 2
        R_W2 = R_M + 8
        R_AN = (R_W2 + NK * 8 + 31) // 32 * 32
        for j in range(2):
            idx_s[j] = R_AN // 32
        cps[0].wait(); cps[1].wait()
        cps[5].start()
        b1 = b1_s[...].astype(f32).reshape(1, F) * SC
        hi = b1.astype(bf16).astype(f32)
        row = lax.broadcasted_iota(jnp.int32, (S, F), 0)
        ext = jnp.where(row == 0, hi, jnp.where(row == 1, b1 - hi, 0.0))
        w1a = jnp.concatenate([ext, w1_s[...].astype(f32), jnp.zeros((128 - 2 * S, F), f32)], axis=0).astype(bf16)
        w1t = w1a.T
        for l_s in lss: l_s[0:R_M, :] = pltpu.bitcast(w1t, u32)
        if V:
            lv = pltpu.bitcast(jnp.concatenate([lss[0][4 * (NG - 1 - p):4 * (NG - p), :] for p in vpos], axis=0), bf16)
            lvf = lv.astype(f32)
            for s in range(XS):
                wb_s[s] = jnp.broadcast_to(lvf[:, S + s:S + s + 1], (8 * V, 128))
            wb_s[S] = jnp.broadcast_to(lvf[:, 0:1] + lvf[:, 1:2], (8 * V, 128))
            r = lax.broadcasted_iota(jnp.int32, (2 * S, (S - XS) * 128), 0)
            c = lax.broadcasted_iota(jnp.int32, (2 * S, (S - XS) * 128), 1)
            sel = jnp.where(r == S + XS + (c >> 7), 1.0, 0.0).astype(bf16)
            wb = jnp.dot(lv[:, :2 * S], sel, preferred_element_type=f32)
            for s in range(XS, S):
                wb_s[s] = wb[:, (s - XS) * 128:(s - XS + 1) * 128]
        cps[2].wait(); cps[3].wait()
        w2u = pltpu.bitcast(w2_s[...], u32)
        for k in range(NK):
            for l_s in lss: l_s[R_W2 + 8 * k:R_W2 + 8 * k + 8, :] = w2u[:, k * FC:(k + 1) * FC]
        m = jnp.dot(w2_s[...], w1t, preferred_element_type=f32)
        b2 = b2_s[...].astype(f32).reshape(1, S) * (SC / 0.5)
        eye = lax.broadcasted_iota(jnp.int32, (S, S), 0) == lax.broadcasted_iota(jnp.int32, (S, S), 1)
        m = m + jnp.concatenate([jnp.where(eye, b2, 0.0), jnp.zeros((S, 128 - S), f32)], axis=1)
        mh = m.astype(bf16).astype(f32)
        m = mh + pltpu.roll(m - mh, 2 * S, 1)
        for l_s in lss: l_s[R_M:R_M + 8, :] = pltpu.bitcast(m.astype(bf16), u32)
        def ln(b0):
            for bb in range(UB):
                x = x_s[b0 + bb].astype(f32)
                mu = jnp.mean(x, axis=-1, keepdims=True)
                xc = x - mu
                var = jnp.mean(xc * xc, axis=-1, keepdims=True)
                hf = xc * (lax.rsqrt(var + 1e-5) * SC)
                hf_s[bb] = hf
                hp_s[bb] = pltpu.bitcast(hf.astype(bf16), u32)
        cps[4].wait()
        ln(0)
        cps[5].wait()
        def body(it, carry):
            slots, pend, aslot = [], [], {}
            def emit(e):
                while pend and len(slots) >= pend[0][0] + DL:
                    slots.append(pend.pop(0)[1])
                slots.append(e)
            for u in range(U):
                for a in range(NA):
                    if a == LP_: emit(('l', u, 0))
                    emit(('a', u, a))
                    aslot[u, a] = len(slots) - 1
                    k0 = mpos[a] // 16
                    k1 = mpos[a + 1] // 16 if a + 1 < NA else NK
                    if k1 > k0: pend.append((len(slots) - 1, ('b', u, k0)))
            slots += [p[1] for p in pend]
            g, front = {}, []
            cnt = [0]
            abase = pl.multiple_of(idx_s[it & 1] * 32, 32)
            def anchor(v):
                lss[now[0] % NL][pl.ds(abase + 8 * (cnt[0] % 16), 8), :] = pltpu.bitcast(v, u32)
                cnt[0] += 1
            now = [0]
            def vpu_all():
                for u in range(U):
                    d0 = (u % NC) * DC
                    for n, p in enumerate(vpos):
                        outs = []
                        for c0 in range(d0, d0 + DC, 128 * CH):
                            z = jnp.concatenate([wb_s[S, 8 * n:8 * n + 8, :]] * CH, axis=1)
                            for s in range(S):
                                wv = jnp.concatenate([wb_s[s, 8 * n:8 * n + 8, :]] * CH, axis=1)
                                z = z + wv * jnp.concatenate([jnp.broadcast_to(hf_s[u // NC, s:s + 1, c:c + 128], (8, 128)) for c in range(c0, c0 + 128 * CH, 128)], axis=1)
                                if s < S - 1: yield z
                            outs.append(act(z))
                            front.append((now[0] + TL, outs[-1]))
                            if len(outs) == NT // CH: g[u, p] = jnp.concatenate(outs, axis=1)
                            yield z
                            yield None
                            yield None
            gen = vpu_all()
            NST = (S + 2) * NT // CH
            wm = WM if isinstance(WM, tuple) else (WM,)
            wts = [1.0 + sum(w - 1.0 for q, w in enumerate(wm) if n < PD + q or slots[n - PD - q][0] != 'a') for n in range(len(slots))]
            target = [0] * len(slots)
            dls = []
            for u in range(U):
                for p in vpos:
                    a = min(sum(q < p for q in mpos), NA - 1)
                    dls.append(min(aslot[u, a] + GP - VD, slots.index(('b', u, p // 16))))
            cw = np.cumsum(wts)
            i0, base_n, base_c = 0, -1, 0
            while i0 < len(dls):
                w0 = cw[base_n] if base_n >= 0 else 0.0
                rates = [((j + 1) * NST - base_c) / (cw[dls[j]] - w0) for j in range(i0, len(dls))]
                j = i0 + int(np.argmax(rates))
                for n in range(base_n + 1, dls[j] + 1):
                    target[n] = base_c + int(round(rates[j - i0] * (cw[n] - w0)))
                base_n, base_c, i0 = dls[j], (j + 1) * NST, j + 1
            done = 0
            ls, accs, due = [], {}, []
            last = None
            ones = jnp.full((8, DC), 0x3F803F80, u32)
            for n, (kind, u, a) in enumerate(slots):
                now[0] = n
                l_s = lss[n % NL]
                while done < target[n]:
                    r = next(gen); done += 1
                    last = r if r is not None else last
                for o in ORD:
                    if o == 'g':
                        for e in [e for e in due if e[0] <= n]:
                            due[:] = [q for q in due if q is not e]
                            for j in range(8):
                                if e[2] >> j & 1: anchor(e[1][8 * (j // 4):8 * (j // 4) + 8, 128 * (j % 4):128 * (j % 4) + 128])
                    while o == 'f' and front and front[0][0] <= n:
                        v = front.pop(0)[1]
                        for j in range(CH): anchor(v[:, 128 * j:128 * j + 128])
                    if o == 'z' and last is not None:
                        for j in range(CH): anchor(last[:, 128 * j:128 * j + 128])
                        last = None
                if kind == 'b':
                    gg = jnp.concatenate([g.pop((u, 16 * a + 15 - q)) for q in range(16)], axis=0)
                    r = R_W2 + 8 * (NK - 1 - a)
                    p = lax.dot_general(pltpu.bitcast(l_s[r:r + 8, :], bf16), gg, DN, preferred_element_type=f32)
                    accs[u] = accs[u] + p
                    if a == NK - 1:
                        accs[u] = accs[u] * (0.5 / SC)
                        o_s[it * UB + u // NC, :, (u % NC) * DC:(u % NC + 1) * DC] = accs[u].astype(o_s.dtype)
                    due.append((n + AP, accs[u], AM))
                    continue
                r = R_M if kind == 'l' else 4 * (NG - 2 - mpos[a])
                ls.append((n, l_s[r:r + 8, :]))
                if n + 1 == len(slots) or slots[n + 1][0] == 'b' or slots[n + 1][1] != u or len(ls) == 9:
                    hh = hp_s[u // NC, :, (u % NC) * DC:(u % NC + 1) * DC]
                    K2 = any(slots[m_][0] == 'l' for m_, _ in ls)
                    hv = pltpu.bitcast(jnp.concatenate([ones, hh] * (1 + K2), axis=0), bf16)
                    lhs = pltpu.bitcast(jnp.concatenate([v for _, v in ls], axis=0), bf16)[:, :hv.shape[0]]
                    w = jnp.dot(lhs, hv, preferred_element_type=f32)
                    for j, (m_, _) in enumerate(ls):
                        if slots[m_][0] == 'l': accs[u] = w[16 * j:16 * j + 16]
                        else:
                            v = act(w[16 * j:16 * j + 16])
                            if HALF:
                                due.append((m_ + GP - 1, v, GM & 15)); due.append((m_ + GP, v, GM & 240))
                            else:
                                due.append((m_ + GP, v, GM))
                            g[u, mpos[slots[m_][2]] + 1] = v[0:8]
                            g[u, mpos[slots[m_][2]]] = v[8:16]
                    ls = []
            ln(jnp.minimum((it + 1) * UB, B - UB))
            pltpu.make_async_copy(o_s.at[pl.ds(it * UB, UB)], o_hbm.at[pl.ds(it * UB, UB)], sem.at[6]).start()
            return carry
        nit = NIT or (B * NC // U)
        lax.fori_loop(0, nit, body, 0)
        pltpu.make_async_copy(o_s.at[0:nit * UB], o_hbm.at[0:nit * UB], sem.at[6]).wait()

    def fn(x, w1, b1, w2, b2):
        B, S, D = x.shape
        F = w1.shape[1]
        UB = U * DC // D
        hbm = pl.BlockSpec(memory_space=pltpu.HBM)
        return pl.pallas_call(
            kern,
            out_shape=jax.ShapeDtypeStruct((B, S, D), x.dtype),
            in_specs=[hbm] * 5, out_specs=hbm,
            scratch_shapes=[pltpu.VMEM(x.shape, bf16), pltpu.VMEM((S, F), bf16), pltpu.VMEM((F,), bf16), pltpu.VMEM((S, F), bf16), pltpu.VMEM((S,), bf16),
                            pltpu.VMEM(x.shape, bf16), pltpu.VMEM((S + 1, 8 * max(V, 1), 128), f32),
                            pltpu.VMEM((UB, S // 2, D), u32), pltpu.VMEM((UB, S, D), f32), pltpu.SMEM((2,), jnp.int32), pltpu.SemaphoreType.DMA((7,))]
                           + [pltpu.VMEM((F // 2 + F // 16 + 256, 128), u32)] * NL,
            compiler_params=pltpu.CompilerParams(flags=flags),
            name="mixer",
        )(x, w1, b1, w2.T, b2)
    return fn


@jax.jit
def pallas_standalone__mixer_token_mlp__sampling_kernel(x, w1, b1, w2, b2):
    return make(U=4, V=32)(x, w1, b1, w2, b2)
```

```python
import jax
import jax.experimental.pallas as pl
import jax.experimental.pallas.tpu as pltpu
import jax.numpy as jnp
import numpy as np
from jax import lax

_C1 = float(np.sqrt(2.0 / np.pi))
_SC = float((_C1 * 0.044715) ** (1.0 / 3.0))
_KK = _C1 / _SC
_EPS = 1e-5

_L = 128
_DC = 512

_PEEL = 1
_UNROLL = 9
_PAIRS = 23
_PHASE = 0.6
_GAP = 6
_MM2_LAG = 11
_ACT_LAG = 12
_ACT_TILE = 5
_ACC_LAG = 12
_ACC_TILE = 7
_VPU_START = -3.0
_VPU_DUE = 0
_VPU_AHEAD = 3
_VPU_ACT_LAG = 3
_VPU_ACT_STEPS = 2
_LULL_LAG = 12
_LULL = (1.5, 1.5)
_UNTIED = 4
_LINEAR_AT = 96
_TAIL_LINEAR = (1, 3, 5, 7)
_NORM_EARLY = (3, 7)
_FIRST_BLOCKS = 6
_T_BLOCK = 1.4
_T_TABLE = (28, 4.1, 0)
_T_NORM = (132, 3.8, 10, 12)

_NN = (((1,), (0,)), ((), ()))
_NT = (((1,), (1,)), ((), ()))


def _dot(a, b, dims=_NN):
    return lax.dot_general(a, b, dims, lax.Precision.DEFAULT, preferred_element_type=jnp.float32)


def _act(w):
    return lax.mul(w, lax.tanh(lax.mul(w, lax.add(lax.mul(w, w), np.float32(_KK)))))


def _vreg(v, j):
    r, c = 8 * (j // 4), _L * (j % 4)
    return lax.slice(v, (r, c), (r + 8, c + _L))


def _add(p, q):
    return [lax.add(a, b) for a, b in zip(p, q)]


def _packed(v):
    return pltpu.bitcast(v, jnp.float32)


def _unpacked(v):
    return pltpu.bitcast(v, jnp.bfloat16)


def _timeline(n_groups, pairs, inline_linear):
    mxu = [p for p in range(n_groups) if not any(p in pair for pair in pairs)][0::2]
    slots, waiting, column_ends = [], [], []

    def emit(slot):
        while waiting and len(slots) >= waiting[0][0] + _MM2_LAG:
            slots.append(waiting.pop(0)[1])
        slots.append(slot)

    for u, inline in enumerate(inline_linear):
        for p, nxt in zip(mxu, mxu[1:] + [n_groups]):
            if inline and p == mxu[_LINEAR_AT]:
                emit(("lin", u, 0))
            emit(("mm1", u, p))
            if nxt // 16 > p // 16:
                waiting.append((len(slots) - 1, ("mm2", u, p // 16)))
        column_ends.append(len(slots) - 1)
    n_stream = len(slots)
    linear = [("lin", u, 0) for u, inline in enumerate(inline_linear) if not inline]
    rest = [slot for _, slot in waiting]
    slots += linear[:1] + rest[:-1] + linear[1:] + rest[-1:]

    busy = lambda n: not 0 <= n < n_stream or slots[n][0] == "mm1"
    clock = np.cumsum([
        1.0 + sum(w - 1.0 for q, w in enumerate(_LULL) if not busy(n - _LULL_LAG - q))
        for n in range(len(slots) + _ACT_LAG)
    ])
    ends = [clock[n + _VPU_DUE] for n in column_ends]
    steps = len(pairs) * (56 + 4 * _VPU_ACT_STEPS + 1) * np.arange(len(ends) + 1)
    steps_due = np.rint(np.interp(clock, [_VPU_START] + ends, steps)).astype(int)
    steps_due[n_stream:] = steps[-1]
    return slots, n_stream, steps_due


def _table_rows(S, F):
    lin = F // 2
    w2 = lin + S // 2
    spare = (w2 + (F // _L) * (S // 2) + 31) // 32 * 32
    return lin, w2, spare, spare + 128, 8 * (7 * (S // 2) + 3)


def _kernel(x_hbm, w1_hbm, b1_hbm, w2t_hbm, b2_hbm, o_hbm,
            x_s, w1_s, b1_s, w2t_s, b2_s, o_s,
            hm_s, hv_s, xf_s, acc_s, stat_s, w1b_s, idx_s, sem, table, wv_s):
    f32, bf16 = jnp.float32, jnp.bfloat16
    B, S, D = x_hbm.shape
    F = w1_hbm.shape[1]
    H = S // 2
    n_blocks, n_groups, n_cols = F // _L, F // 8, B * (D // _DC)
    n_iter = (n_cols - _PEEL) // _UNROLL
    b_first = (_PEEL + 1) // 2
    r_lin, r_w2, r_spare, r_vpu, pair_rows = _table_rows(S, F)
    n_mm1 = n_groups // 2 - _PAIRS
    pairs = [2 * int((2 * j + _PHASE) * n_mm1 / (2 * _PAIRS)) + 2 * j for j in range(_PAIRS)]
    pairs = [(p, p + _GAP + 1) for p in pairs]

    def vpu_weights(j, r):
        if r % _UNTIED == 2:
            return wv_s, pl.ds(j * pair_rows + 8 * r, 8)
        return table, pl.ds(r_vpu + j * pair_rows + 8 * r, 8)

    loads = [
        pltpu.make_async_copy(src, dst, sem.at[i])
        for i, (src, dst) in enumerate([
            (x_hbm.at[0:b_first], x_s.at[0:b_first]),
            (w1_hbm, w1_s), (b1_hbm, b1_s), (w2t_hbm, w2t_s), (b2_hbm, b2_s),
            (x_hbm.at[b_first:B], x_s.at[b_first:B]),
        ])
    ]
    for copy in loads[:5]:
        copy.start()

    idx_s[0] = 0
    idx_s[1] = r_spare // 32
    recent = []

    def lanes(col):
        return pl.ds(pl.multiple_of((col & 1) * _DC, _DC), _DC)

    def norm_mean(b):
        if recent:
            x_s[B + idx_s[0], :, 0:_L] = _unpacked(recent[0])
        x = x_s[b].astype(f32)
        xf_s[b] = x
        stat_s[0, b] = jnp.broadcast_to(jnp.mean(x, axis=-1, keepdims=True), (S, _L))

    def norm_scale(b):
        x = xf_s[b + idx_s[0] if recent else b]
        xc = x - jnp.concatenate([stat_s[0, b]] * (D // _L), axis=1)
        var = jnp.mean(xc * xc, axis=-1, keepdims=True)
        scale = jnp.broadcast_to(lax.rsqrt(var + _EPS) * _SC, (S, _L))
        stat_s[1, b] = scale
        return [(_T_NORM[3], scale[:H]), (_T_NORM[3], scale[H:])]

    def norm_apply(col, u):
        b = col >> 1
        mean, scale = (jnp.concatenate([stat_s[i, b]] * (_DC // _L), axis=1) for i in range(2))
        h = (xf_s[b, :, lanes(col)] - mean) * scale
        hm_s[u, H:S] = _packed(h.astype(bf16))
        b11, b12 = h[:H, :_DC // 2], h[:H, _DC // 2:]
        b21, b22 = h[H:, :_DC // 2], h[H:, _DC // 2:]
        t1 = b12 - b11
        t2 = b22 - t1
        hv_s[u] = jnp.concatenate([b11, b21, b22, b21 - t2, t1, t2, b22 - b12], axis=0)

    def finish(col, acc):
        o_s[col >> 1, :, lanes(col)] = (acc * (0.5 / _SC)).astype(o_s.dtype)

    def run_columns(col0, pairs, inline_linear, chores):
        slots, n_stream, steps_due = _timeline(n_groups, pairs, inline_linear)
        last = len(inline_linear) - 1
        spare = pl.multiple_of(idx_s[1] * 32, 32)
        spare = [spare + 8 * j for j in range(16)]
        act, ties, horizon = {}, [], [0]

        def vpu_pair(u, j):
            def weights(r):
                ref, rows = vpu_weights(j, r)
                return ref[rows, :]

            def product(i, acc, pause_last=True):
                for r in range(i * H, (i + 1) * H):
                    w = weights(r)
                    terms = [
                        lax.mul(w, lax.broadcast_in_dim(hv_s[u, r:r + 1, c:c + _L], (8, _L), (0, 1)))
                        for c in (0, _L)
                    ]
                    acc = terms if acc is None else _add(acc, terms)
                    if pause_last or r + 1 < (i + 1) * H:
                        yield
                return acc

            def activate(ws):
                out = [_act(w) for w in ws]
                ties.extend((horizon[0] + _VPU_ACT_LAG, 0, v) for v in out)
                return out

            u1 = yield from product(0, [weights(7 * H)] * 2)
            c11 = activate((yield from product(1, u1, False)))
            yield from range(_VPU_ACT_STEPS + 1)
            u2 = yield from product(5, u1)
            p5 = yield from product(4, None)
            c12 = activate((yield from product(2, _add(u2, p5), False)))
            act[u, pairs[j][0]] = lax.concatenate(c11 + c12, 1)
            yield from range(_VPU_ACT_STEPS + 2)
            u3 = yield from product(6, _add(u2, [weights(7 * H + 1)] * 2), False)
            c22 = activate(_add(u3, p5))
            yield from range(_VPU_ACT_STEPS + 1)
            c21 = activate((yield from product(3, u3, False)))
            act[u, pairs[j][1]] = lax.concatenate(c21 + c22, 1)
            yield from range(_VPU_ACT_STEPS + 1)

        vpu = (s for u in range(last + 1) for j in range(len(pairs)) for s in vpu_pair(u, j))
        steps = n_ties = 0
        lhs, acc = [], {}
        for n, (kind, u, pos) in enumerate(slots):
            while chores and chores[0][0] <= n:
                ties.extend((n + lag, 3, v) for lag, v in chores.pop(0)[1]() or ())
            while horizon[0] <= n + _VPU_AHEAD:
                while steps < steps_due[horizon[0]]:
                    next(vpu)
                    steps += 1
                horizon[0] += 1
            for _, rank, v in sorted((t for t in ties if t[0] <= n < n_stream), key=lambda t: t[1]):
                table[pl.ds(spare[n_ties % 16], 8), :] = v
                n_ties += 1
                if rank == 1:
                    recent[:] = [v]
            ties[:] = [t for t in ties if t[0] > n]

            if kind == "mm2":
                r = r_w2 + H * (n_blocks - 1 - pos)
                g = lax.concatenate([act.pop((u, 16 * pos + 15 - q)) for q in range(16)], 0)
                y = _dot(_unpacked(table[r:r + H, :]), g)
                acc[u] = lax.add(acc[u], y) if u in acc else y
                ties.append((n + _ACC_LAG, 2, _vreg(acc[u], _ACC_TILE)))
                if pos == n_blocks - 1:
                    if inline_linear[u] or u == last:
                        finish(col0 + u, acc.pop(u))
                    else:
                        acc_s[u] = acc.pop(u)
                continue

            r = r_lin if kind == "lin" else 4 * (n_groups - 2 - pos)
            lhs.append((n, table[r:r + 8, :]))
            if slots[n + 1][0] != "mm2" and slots[n + 1][1] == u and len(lhs) < 9 and n + 1 < n_stream:
                continue
            rhs = hm_s[u]
            if any(slots[m][0] == "lin" for m, _ in lhs):
                rhs = lax.concatenate([rhs, rhs], 0)
            rhs = _unpacked(rhs)
            rows = _unpacked(lax.concatenate([v for _, v in lhs], 0))[:, :rhs.shape[0]]
            w = _dot(rows, rhs)
            for i, (m, _) in enumerate(lhs):
                v = lax.slice(w, (16 * i, 0), (16 * i + 16, _DC))
                if slots[m][0] == "mm1":
                    newest = _act(v)
                    ties.append((m + _ACT_LAG, 1, _vreg(newest, _ACT_TILE)))
                    if m < n_stream - _NORM_EARLY[1]:
                        early = newest
                    act[u, slots[m][2] + 1] = lax.slice(newest, (0, 0), (8, _DC))
                    act[u, slots[m][2]] = lax.slice(newest, (8, 0), (16, _DC))
                elif inline_linear[u] or u == last:
                    acc[u] = lax.add(acc[u], v) if u in acc else v
                else:
                    finish(col0 + u, acc_s[u + idx_s[0]] + v)
            lhs = []
        for _, chore in chores:
            chore()

        for u in range(_UNROLL):
            if u == 0:
                xf_s[B + idx_s[0], 0:8, 0:_L] = _vreg(early, 7)
            if u == _NORM_EARLY[0]:
                xf_s[B + idx_s[0], :, _DC:2 * _DC] = newest
            norm_apply(jnp.minimum(col0 + last + 1 + u, n_cols - 1), u)

    for u in range(hm_s.shape[0]):
        hm_s[u, 0:H] = _packed(jnp.ones((S, _DC), bf16))
    loads[0].wait()
    loads[5].start()
    for b in range(b_first):
        norm_mean(b)
        norm_scale(b)
    for u in range(_PEEL):
        norm_apply(u, u)
    loads[1].wait()
    loads[2].wait()

    b1 = b1_s[...].astype(f32).reshape(1, F) * _SC
    b1_hi = b1.astype(bf16).astype(f32)
    row = lax.broadcasted_iota(jnp.int32, (S, F), 0)
    bias = jnp.where(row == 0, b1_hi, jnp.where(row == 1, b1 - b1_hi, 0.0)).astype(bf16)
    w1b = jnp.concatenate([_packed(bias), _packed(w1_s[...])], axis=0)
    w1b_s[...] = w1b

    def store_linear():
        table[r_lin:r_lin + H, :] = _packed(lin.astype(bf16))

    def store_block(k):
        cols = slice(k * _L, (k + 1) * _L)
        block = jnp.concatenate([w1b_s[:, cols], jnp.zeros((_L // 2 - S, _L), f32)], axis=0)
        table[k * _L // 2:(k + 1) * _L // 2, :] = _packed(_unpacked(block).T)

    for i in range(_FIRST_BLOCKS):
        store_block(n_blocks - 1 - i)

    loads[3].wait()
    loads[4].wait()
    for k in range(n_blocks):
        table[r_w2 + H * k:r_w2 + H * (k + 1), :] = _packed(w2t_s[:, k * _L:(k + 1) * _L])
    lin = _dot(w2t_s[...], _unpacked(w1b), _NT)
    b2 = b2_s[...].astype(f32).reshape(1, S) * (_SC / 0.5)
    eye = lax.broadcasted_iota(jnp.int32, (S, S), 0) == lax.broadcasted_iota(jnp.int32, (S, S), 1)
    lin = lin + jnp.concatenate([jnp.where(eye, b2, 0.0), jnp.zeros((S, S), f32)], axis=1)
    lin_hi = lin.astype(bf16).astype(f32)
    lin = jnp.concatenate([lin_hi, lin - lin_hi, jnp.zeros((S, _L - 4 * S), f32)], axis=1)

    pair_w = {}

    def load_pair(j):
        rows = [table[4 * (n_groups - 1 - p):4 * (n_groups - p), :] for p in pairs[j]]
        pair_w[j] = _unpacked(jnp.concatenate(rows, axis=0)).astype(f32)

    def store_pair(j, s):
        spread = lambda c: jnp.broadcast_to(pair_w[j][:, c:c + 1], (16, _L))
        if s < H:
            lo, up = spread(S + s), spread(S + H + s)
            a11, a21, a12, a22 = lo[:8], lo[8:], up[:8], up[8:]
            s1 = a21 + a22
            s2 = s1 - a11
            out = [(i * H + s, v) for i, v in enumerate((a11, a12, a12 - s2, a22, s1, s2, a11 - a21))]
        else:
            b = spread(0) + spread(1)
            out = [(7 * H, b[:8]), (7 * H + 1, b[8:] - b[:8])]
        for r, v in out:
            ref, rows = vpu_weights(j, r)
            ref[rows, :] = v
        return [(_T_TABLE[2], out[2][1])] if ref is wv_s else None

    chores = [(_T_BLOCK * i, lambda k=n_blocks - 1 - i: store_block(k))
              for i in range(_FIRST_BLOCKS, n_blocks)]
    chores.append((20, store_linear))
    for j in range(_PAIRS):
        t = _T_TABLE[0] + _T_TABLE[1] * j
        assert t >= _T_BLOCK * (pairs[j][1] // 16)
        chores.append((t, lambda j=j: load_pair(j)))
        for s in range(H + 1):
            chores.append((t + 9 + _T_TABLE[1] * s / (H + 1), lambda j=j, s=s: store_pair(j, s)))
    chores.append((_T_NORM[0], loads[5].wait))
    for b in range(b_first, B):
        t = _T_NORM[0] + _T_NORM[1] * (b - b_first)
        chores += [(t, lambda b=b: norm_mean(b)), (t + _T_NORM[2], lambda b=b: norm_scale(b))]
    chores.sort(key=lambda chore: chore[0])
    run_columns(0, [], [False] * _PEEL, chores)

    done = (n_cols - _UNROLL) // (D // _DC)
    stores = [
        pltpu.make_async_copy(o_s.at[lo:hi], o_hbm.at[lo:hi], sem.at[6 + i])
        for i, (lo, hi) in enumerate([(0, done), (done, B)])
    ]

    def body(it, carry):
        pl.when(it == n_iter - 1)(stores[0].start)
        inline = [u not in _TAIL_LINEAR for u in range(_UNROLL)]
        run_columns(_PEEL + it * _UNROLL, pairs, inline, [])
        return carry

    lax.fori_loop(0, n_iter, body, 0)
    stores[1].start()
    for copy in stores:
        copy.wait()


@jax.jit
def pallas_standalone__mixer_token_mlp__sampling_kernel(
    x: jax.Array,
    w1: jax.Array,
    b1: jax.Array,
    w2: jax.Array,
    b2: jax.Array,
):
    B, S, D = x.shape
    F = w1.shape[1]
    assert S == 16 and D == 2 * _DC and F % _L == 0 and (2 * B - _PEEL) % _UNROLL == 0
    f32, bf16 = jnp.float32, jnp.bfloat16
    n_slots = max(_PEEL, _UNROLL)
    *_, r_vpu, pair_rows = _table_rows(S, F)
    hbm = pl.BlockSpec(memory_space=pltpu.HBM)
    return pl.pallas_call(
        _kernel,
        out_shape=jax.ShapeDtypeStruct((B, S, D), x.dtype),
        in_specs=[hbm] * 5,
        out_specs=hbm,
        scratch_shapes=[
            pltpu.VMEM((B + 1, S, D), bf16),
            pltpu.VMEM((S, F), bf16),
            pltpu.VMEM((F,), bf16),
            pltpu.VMEM((S, F), bf16),
            pltpu.VMEM((S,), bf16),
            pltpu.VMEM((B, S, D), bf16),
            pltpu.VMEM((n_slots, S, _DC), f32),
            pltpu.VMEM((n_slots, 7 * S // 2, _DC // 2), f32),
            pltpu.VMEM((B + 1, S, D), f32),
            pltpu.VMEM((n_slots, S, _DC), f32),
            pltpu.VMEM((2, B, S, _L), f32),
            pltpu.VMEM((S, F), f32),
            pltpu.SMEM((2,), jnp.int32),
            pltpu.SemaphoreType.DMA((8,)),
            pltpu.VMEM((r_vpu + _PAIRS * pair_rows, _L), f32),
            pltpu.VMEM((_PAIRS * pair_rows, _L), f32),
        ],
        compiler_params=pltpu.CompilerParams(vmem_limit_bytes=48 * 1024 * 1024),
        name="mixer_token_mlp",
    )(x, w1, b1, w2.T, b2)
```
